```python
import os as _os
_os.environ.setdefault("JAX_PLATFORMS", "cpu")
import jax
import jax.numpy as jnp

def _softmax(x, axis=-1):
    return jax.nn.softmax(x, axis=axis)
def _gelu(x):
    return jax.nn.gelu(x, approximate=True)
def _silu(x):
    return jax.nn.silu(x)
def _sigmoid(x):
    return jax.nn.sigmoid(x)
def _layernorm(x, axis=-1, eps=1e-5):
    m = jnp.mean(x, axis=axis, keepdims=True)
    v = jnp.var(x, axis=axis, keepdims=True)
    return (x - m) / jnp.sqrt(v + eps)
def _scatter_add(tgt, idx, src, axis=0):
    return tgt.at[idx].add(src)
def _segment_sum(src, seg, n):
    return jax.ops.segment_sum(src, seg, n)
class _Rng:
    def __init__(self, key):
        self._k = key
    def _next(self):
        self._k, sub = jax.random.split(self._k)
        return sub
    def normal(self, shape):
        return jax.random.normal(self._next(), shape, dtype=jnp.bfloat16)
    def randint(self, lo, hi, shape):
        return jax.random.randint(self._next(), shape, lo, hi, dtype=jnp.int32)
    def uniform(self, shape, lo=0.0, hi=1.0):
        return jax.random.uniform(self._next(), shape, jnp.bfloat16, lo, hi)
    def permutation(self, n):
        return jax.random.permutation(self._next(), n)


kernel_name = 'gated_mix__mha_block__mixer_s_mlp__prompt'

def setup_inputs():
    _rng = _Rng(jax.random.key(int.from_bytes(__import__("os").urandom(4), "little")))
    _w = (lambda a: (lambda t: t.astype(jnp.bfloat16) if jnp.issubdtype(t.dtype, jnp.floating) else t)(jnp.asarray(a)))
    def _A_setup():
        B, S, D, H = 1, 2048, 512, 32
        return {
            "x": _w((lambda *s: _rng.normal(s) * 0.05)(B, S, D)),
            "wqkv": _w((lambda *s: _rng.normal(s) * 0.8)(D, 3 * D)),
            "wo": _w((lambda *s: _rng.normal(s) * 0.05)(D, D)),
        }
    _A_in = _A_setup()

    def _B_setup():
        B, S, D, F = 1, 2048, 512, 1792
        return {
            "x":  _w((lambda *s: _rng.normal(s) * 0.05)(B, S, D)),
            "w1": _w((lambda *s: _rng.normal(s) * 0.2)(D, D) * (D ** -0.5)),
            "w2": _w((lambda *s: _rng.normal(s) * 0.2)(D, D) * (D ** -0.5)),
            "w3": _w((lambda *s: _rng.normal(s) * 0.2)(D, F) * (D ** -0.5)),
            "w4": _w((lambda *s: _rng.normal(s) * 0.2)(F, D) * (F ** -0.5)),
        }
    _B_in = _B_setup()

    return {
        "A_x": _A_in["x"],
        "A_wqkv": _A_in["wqkv"],
        "A_wo": _A_in["wo"],
        "B_x": _B_in["x"],
        "B_w1": _B_in["w1"],
        "B_w2": _B_in["w2"],
        "B_w3": _B_in["w3"],
        "B_w4": _B_in["w4"],
        "gate_w": _w((lambda *s: _rng.normal(s) * 0.05)(512) * 16.0),
    }

def reference(A_x, A_wqkv, A_wo, B_x, B_w1, B_w2, B_w3, B_w4, gate_w):
    def _A_ref(x, wqkv, wo):
        B, S, D = x.shape
        H = 32
        Dh = D // H
        qkv = (lambda x, *d: x.transpose(*d))((x @ wqkv).reshape(B, S, 3, H, Dh), 2, 0, 3, 1, 4)
        q, k, v = qkv[0], qkv[1], qkv[2]
        scores = jnp.einsum("bhqd,bhkd->bhqk", q, k) * (Dh ** -0.5)
        p = _softmax(scores, axis=-1)
        o = jnp.einsum("bhqk,bhkd->bhqd", p, v)
        return (lambda x, *d: x.transpose(*d))(o, 0, 2, 1, 3).reshape(B, S, D) @ wo

    def _B_ref(x, w1, w2, w3, w4):
        B, S, D = x.shape
        h = _gelu(_layernorm(x, axis=-1) @ w1)
        c = D // 4
        g0 = jnp.pad(h[:, :, 0*c:1*c], ((0, 0), (1, 0), (0, 0)))[:, :S, :]
        g1 = jnp.pad(h[:, :, 1*c:2*c], ((0, 0), (0, 1), (0, 0)))[:, 1:, :]
        g2 = jnp.pad(h[:, :, 2*c:3*c], ((0, 0), (2, 0), (0, 0)))[:, :S, :]
        g3 = jnp.pad(h[:, :, 3*c:   ], ((0, 0), (0, 2), (0, 0)))[:, 2:, :]
        hs = jnp.concatenate([g0, g1, g2, g3], axis=-1) @ w2
        x1 = x + hs
        h2 = _gelu(_layernorm(x1, axis=-1) @ w3) @ w4
        return x1 + h2

    x = A_x
    g = _sigmoid((x * gate_w).sum(-1, keepdims=True))
    a = _A_ref(x, A_wqkv, A_wo)
    b = _B_ref(x, B_w1, B_w2, B_w3, B_w4)
    return g * a + (1 - g) * b
```

```python
import math

import jax
import jax.numpy as jnp
import jax.experimental.pallas as pl
import jax.experimental.pallas.tpu as pltpu

_H = 32
_NQ = 512
_KB = 128
_RB = 512
_HALO = 8
_EPS = 1e-5
_LOG2E = 1.4426950408889634
_L_HI = 2.0 ** 40
_L_LO = 2.0 ** -40

_F32 = jnp.float32
_BF16 = jnp.bfloat16


def _dot(a, b):
    return jnp.dot(a, b, preferred_element_type=_F32)


def _dot_nt(a, b):
    return jax.lax.dot_general(a, b, (((1,), (1,)), ((), ())), preferred_element_type=_F32)


def _dot_tn(a, b):
    return jax.lax.dot_general(a, b, (((0,), (0,)), ((), ())), preferred_element_type=_F32)


def _gelu(x):
    c = math.sqrt(2.0 / math.pi)
    return (0.5 * x) * (1.0 + jnp.tanh(x * (c + (c * 0.044715) * (x * x))))


def _layernorm(x):
    m = jnp.mean(x, axis=-1, keepdims=True)
    d = x - m
    v = jnp.mean(d * d, axis=-1, keepdims=True)
    return d * jax.lax.rsqrt(v + _EPS)


def _kernel(ax_hbm, wqkv_hbm, wo_hbm, w1_hbm, w2_hbm, w3_hbm, w4_hbm, gw_hbm, out_hbm,
            ax, wqkv, wo, w1, w2, w3, w4, gw, outv,
            hbuf, bbuf, wqvt, kbuf, qt, vt, ot, p0, p1, l0, l1, sems, osems):
    S, D = ax.shape
    F = w3.shape[1]
    Dh = D // _H
    nrb = S // _RB
    nqb = S // _NQ
    nkb = S // _KB
    nunits = _H * nqb

    def cp(src, dst, i):
        return pltpu.make_async_copy(src, dst, sems.at[i])

    c_w1 = cp(w1_hbm, w1, 1)
    c_w2 = cp(w2_hbm, w2, 2)
    c_w3 = cp(w3_hbm, w3, 3)
    c_w4 = cp(w4_hbm, w4, 4)
    c_ax = cp(ax_hbm, ax, 0)
    c_wqkv = cp(wqkv_hbm, wqkv, 6)
    c_wo = cp(wo_hbm, wo, 7)
    c_gw = cp(gw_hbm, gw, 5)
    c_ax.start()
    c_w1.start()
    c_ax.wait()
    c_w1.wait()
    for c in (c_w2, c_w3, c_w4, c_wqkv, c_wo, c_gw):
        c.start()

    def rows(i):
        return pl.ds(pl.multiple_of(i * _RB, _RB), _RB)

    hbuf[0:_HALO, :] = jnp.zeros((_HALO, D), _F32)
    hbuf[_HALO + S:, :] = jnp.zeros((_HALO, D), _F32)

    def b1(i, c):
        xn = _layernorm(ax[rows(i), :].astype(_F32)).astype(_BF16)
        hbuf[pl.ds(pl.multiple_of(i * _RB + _HALO, 8), _RB), :] = _gelu(_dot(xn, w1[...]))
        return c

    jax.lax.fori_loop(0, nrb, b1, 0)
    c_w2.wait()
    c_w3.wait()
    c_w4.wait()

    def b2(i, c):
        q = D // 4
        win = pl.ds(pl.multiple_of(i * _RB, _RB), _RB + 2 * _HALO)
        parts = []
        for g, sh in enumerate((1, -1, 2, -2)):
            hw = hbuf[win, g * q:(g + 1) * q]
            parts.append(hw[_HALO - sh:_HALO - sh + _RB].astype(_BF16))
        x1 = ax[rows(i), :].astype(_F32) + _dot(jnp.concatenate(parts, axis=1), w2[...])
        xn = _layernorm(x1).astype(_BF16)
        h = _gelu(_dot(xn, w3[...])).astype(_BF16)
        bbuf[rows(i), :] = x1 + _dot(h, w4[...])
        return c

    jax.lax.fori_loop(0, nrb, b2, 0)

    c_wqkv.wait()
    c_wo.wait()
    c_gw.wait()
    wqvt[0:D, :] = wqkv[:, 0:D].astype(_F32).T.astype(_BF16)
    wqvt[D:2 * D, :] = wqkv[:, 2 * D:3 * D].astype(_F32).T.astype(_BF16)

    def proj(i, c):
        x = ax[rows(i), :]
        k = _dot(x, wqkv[:, D:2 * D]).astype(_BF16)
        for t in range(D // 128):
            kbuf[t, rows(i), :] = k[:, t * 128:(t + 1) * 128]
        qv = _dot_nt(wqvt[...], x)
        qt[i] = (qv[0:D] * (Dh ** -0.5 * _LOG2E)).astype(_BF16)
        v = qv[D:2 * D].astype(_BF16)
        for j in range(_RB // _KB):
            vt[i * (_RB // _KB) + j] = v[:, j * _KB:(j + 1) * _KB]
        return c

    jax.lax.fori_loop(0, nrb, proj, 0)

    hpt = 128 // Dh

    def q_weights(u):
        h = u // nqb
        t = h // hpt
        w = qt[u % nqb, pl.ds(pl.multiple_of(t * 128, 128), 128), :]
        own = jax.lax.broadcasted_iota(jnp.int32, w.shape, 0) // Dh == h % hpt
        return t, jnp.where(own, w, jnp.zeros_like(w))

    def head_rows(u):
        return pl.ds(pl.multiple_of((u // nqb) * Dh, Dh), Dh)

    def step(un, pn, ln, uc, pc, lc, rng):
        if un is not None:
            t, w = q_weights(un)
            l = jnp.zeros((8, _NQ), _F32)
        if uc is not None:
            hr = head_rows(uc)
            acc = jnp.zeros((Dh, _NQ), _F32)
        for kb in range(nkb):
            sl = slice(kb * _KB, (kb + 1) * _KB)
            if uc is not None:
                acc = acc + _dot(vt[kb, hr, :], pc[sl, :])
            if un is not None:
                p = jnp.exp2(_dot(kbuf[t, sl, :], w))
                l = l + jnp.sum(p.reshape(_KB // 8, 8, _NQ), axis=0)
                pn[sl, :] = p.astype(_BF16)
        if un is not None:
            ln[...] = l
        if uc is not None:
            den = jnp.sum(lc[...], axis=0, keepdims=True)
            ot[uc % nqb, hr, :] = (acc / den).astype(_BF16)
            bad = jnp.where((den >= _L_LO) & (den <= _L_HI), 0.0, 1.0)
            rng = jnp.maximum(rng, bad)
        return rng

    flag = jnp.zeros((1, _NQ), _F32)
    flag = step(0, p0, l0, None, None, None, flag)

    def pair(i, flag):
        flag = step(2 * i + 1, p1, l1, 2 * i, p0, l0, flag)
        return step(2 * i + 2, p0, l0, 2 * i + 1, p1, l1, flag)

    flag = jax.lax.fori_loop(0, nunits // 2 - 1, pair, flag)
    flag = step(nunits - 1, p1, l1, nunits - 2, p0, l0, flag)
    flag = step(None, None, None, nunits - 1, p1, l1, flag)

    @pl.when(jnp.max(flag) > 0.0)
    def _():
        def unit(u, c):
            t, w = q_weights(u)
            hr = head_rows(u)

            def scores(kb):
                return _dot(kbuf[t, pl.ds(pl.multiple_of(kb * _KB, _KB), _KB), :], w)

            m = jax.lax.fori_loop(
                0, nkb, lambda kb, m: jnp.maximum(m, jnp.max(scores(kb), axis=0, keepdims=True)),
                jnp.full((1, _NQ), -jnp.inf, _F32))

            def accum(kb, carry):
                den, acc = carry
                p = jnp.exp2(scores(kb) - m)
                return (den + jnp.sum(p, axis=0, keepdims=True),
                        acc + _dot(vt[kb, hr, :], p.astype(_BF16)))

            den, acc = jax.lax.fori_loop(
                0, nkb, accum, (jnp.zeros((1, _NQ), _F32), jnp.zeros((Dh, _NQ), _F32)))
            ot[u % nqb, hr, :] = (acc / den).astype(_BF16)
            return c

        jax.lax.fori_loop(0, nunits, unit, 0)

    def out_copy(i):
        r = slice(i * _NQ, (i + 1) * _NQ)
        return pltpu.make_async_copy(outv.at[r], out_hbm.at[r], osems.at[i])

    for i in range(nqb):
        r = slice(i * _NQ, (i + 1) * _NQ)
        a = _dot_tn(ot[i], wo[...])
        z = jnp.sum(ax[r, :].astype(_F32) * gw[...].astype(_F32), axis=-1, keepdims=True)
        g = 1.0 / (1.0 + jnp.exp(-z))
        outv[r, :] = (g * a + (1.0 - g) * bbuf[r, :]).astype(outv.dtype)
        out_copy(i).start()
    for i in range(nqb):
        out_copy(i).wait()


@jax.jit
def pallas_gated_mix__mha_block__mixer_s_mlp__prompt_kernel(
    A_x: jax.Array,
    A_wqkv: jax.Array,
    A_wo: jax.Array,
    B_x: jax.Array,
    B_w1: jax.Array,
    B_w2: jax.Array,
    B_w3: jax.Array,
    B_w4: jax.Array,
    gate_w: jax.Array,
):
    B, S, D = A_x.shape
    F = B_w3.shape[1]
    assert B == 1
    Dh = D // _H
    vm = pltpu.VMEM
    scratch = [
        vm((S, D), _BF16), vm((D, 3 * D), _BF16), vm((D, D), _BF16),
        vm((D, D), _BF16), vm((D, D), _BF16),
        vm((D, F), _BF16), vm((F, D), _BF16), vm((1, D), _BF16),
        vm((S, D), A_x.dtype),
        vm((S + 2 * _HALO, D), _F32),
        vm((S, D), _F32),
        vm((2 * D, D), _BF16),
        vm((D // 128, S, 128), _BF16),
        vm((S // _NQ, D, _NQ), _BF16),
        vm((S // _KB, D, _KB), _BF16),
        vm((S // _NQ, D, _NQ), _BF16),
        vm((S, _NQ), _BF16), vm((S, _NQ), _BF16),
        vm((8, _NQ), _F32), vm((8, _NQ), _F32),
        pltpu.SemaphoreType.DMA((8,)),
        pltpu.SemaphoreType.DMA((S // _NQ,)),
    ]
    out = pl.pallas_call(
        _kernel,
        out_shape=jax.ShapeDtypeStruct((S, D), A_x.dtype),
        in_specs=[pl.BlockSpec(memory_space=pl.ANY)] * 8,
        out_specs=pl.BlockSpec(memory_space=pl.ANY),
        scratch_shapes=scratch,
        compiler_params=pltpu.CompilerParams(vmem_limit_bytes=96 * 1024 * 1024),
    )(A_x.reshape(S, D), A_wqkv, A_wo, B_w1, B_w2, B_w3, B_w4,
      gate_w.reshape(1, D))
    return out.reshape(B, S, D)
```

```python
import math

import jax
import jax.numpy as jnp
import jax.experimental.pallas as pl
import jax.experimental.pallas.tpu as pltpu

_H = 32
_NQ = 512
_KB = 128
_RB = 512
_HALO = 8
_NV = 16
_RS = 64
_LAG = 4
_HU = 2
_ZQ = 4
_FC = 256
_LC = 128
_EPS = 1e-5
_LOG2E = 1.4426950408889634
_L_HI = 2.0 ** 40
_L_LO = 2.0 ** -40

_F32 = jnp.float32
_BF16 = jnp.bfloat16
_I32 = jnp.int32


def _dot(a, b):
    return jnp.dot(a, b, preferred_element_type=_F32)


def _dot_nt(a, b):
    return jax.lax.dot_general(a, b, (((1,), (1,)), ((), ())), preferred_element_type=_F32)


def _dot_tn(a, b):
    return jax.lax.dot_general(a, b, (((0,), (0,)), ((), ())), preferred_element_type=_F32)


def _pack(x):
    return pltpu.bitcast(x.astype(_BF16), jnp.int32)


def _unpack(x):
    return pltpu.bitcast(x, _BF16)


def _gelu(x):
    c = math.sqrt(2.0 / math.pi)
    return (0.5 * x) * (1.0 + jnp.tanh(x * (c + (c * 0.044715) * (x * x))))


def _layernorm(x):
    m = jnp.mean(x, axis=-1, keepdims=True)
    d = x - m
    v = jnp.mean(d * d, axis=-1, keepdims=True)
    return d * jax.lax.rsqrt(v + _EPS)


def _kernel(ax_hbm, wqkv_hbm, wo_hbm, w1_hbm, w2_hbm, w3_hbm, w4_hbm, gw_hbm, out_hbm,
            ax, wq, wk, wv, wo, w1, w2, w3, w4, gw,
            hbuf, bbuf, gbuf, wqt, wvt, kbuf, kvf, krot, kbr, qt, qf, vt, ot, pb, accb, lb, zero, sems, xsems, osems):
    S, D = ax.shape
    Dh = D // _H
    nrb = S // _RB
    nqb = S // _NQ
    nkb = S // _KB
    vset = [int((i + 0.5) * (S // 16) / _NV) for i in range(_NV)]
    hpt = 128 // Dh

    def rows(i):
        return pl.ds(pl.multiple_of(i * _RB, _RB), _RB)

    def cp(src, dst, i):
        return pltpu.make_async_copy(src, dst, sems.at[i])

    def x_copy(i):
        return pltpu.make_async_copy(ax_hbm.at[rows(i)], ax.at[rows(i)], xsems.at[i])

    c_wk = cp(wqkv_hbm.at[:, D:2 * D], wk, 0)
    c_wq = cp(wqkv_hbm.at[:, 0:D], wq, 1)
    c_wv = cp(wqkv_hbm.at[:, 2 * D:3 * D], wv, 2)
    c_w1 = cp(w1_hbm, w1, 3)
    c_gw = cp(gw_hbm, gw, 4)
    c_w2 = cp(w2_hbm, w2, 5)
    c_w3 = cp(w3_hbm, w3, 6)
    c_w4 = cp(w4_hbm, w4, 7)
    c_wo = cp(wo_hbm, wo, 8)

    x_copy(0).start()
    c_gw.start()
    c_wk.start()
    hbuf[0:_HALO, :] = jnp.zeros((_HALO, D), _F32)
    hbuf[_HALO + S:, :] = jnp.zeros((_HALO, D), _F32)
    for i in range(zero.shape[0]):
        zero[i] = 0
    pb[...] = jnp.zeros(pb.shape, pb.dtype)
    accb[...] = jnp.zeros(accb.shape, accb.dtype)
    lb[...] = jnp.ones(lb.shape, lb.dtype)
    c_gw.wait()
    x_copy(0).wait()
    x_copy(1).start()
    c_w1.start()
    c_wk.wait()

    def blk(i):
        return slice(i * _RB, (i + 1) * _RB)

    def k_proj(i):
        k = _dot(ax[blk(i), :], wk[...])
        for t in range(D // 128):
            kbuf[t, blk(i), :] = k[:, t * 128:(t + 1) * 128].astype(_BF16)
        for n, g in enumerate(vset):
            if i * _RB <= g * 16 < (i + 1) * _RB:
                kg = k[g * 16 - i * _RB:g * 16 + 16 - i * _RB]
                for t in range(D // 128):
                    kvf[t, n * 16:n * 16 + 16, :] = kg[:, t * 128:(t + 1) * 128]

    def norm_gate(i):
        xf = ax[blk(i), :].astype(_F32)
        z = jnp.sum(xf * gw[...].astype(_F32).reshape(1, D), axis=-1, keepdims=True)
        gbuf[blk(i), :] = jnp.broadcast_to(1.0 / (1.0 + jnp.exp(-z)), (_RB, 128))
        return _layernorm(xf).astype(_BF16)

    def mix_in(i, xn):
        hbuf[_HALO + i * _RB:_HALO + (i + 1) * _RB, :] = _gelu(_dot(xn, w1[...]))

    def norm_and_k(i):
        xn = norm_gate(i)
        k_proj(i)
        return xn

    xn = norm_and_k(0)
    x_copy(1).wait()
    for i in range(2, nrb):
        x_copy(i).start()
    for c in (c_wq, c_wv, c_w2):
        c.start()
    c_w1.wait()
    mix_in(0, xn)
    mix_in(1, norm_and_k(1))
    for i in range(2, nrb):
        x_copy(i).wait()
    c_wq.wait()
    for c in (c_w3, c_w4, c_wo):
        c.start()
    c_wv.wait()
    wqt[...] = wq[...].T
    wvt[...] = wv[...].T
    for i in range(2, nrb):
        mix_in(i, norm_and_k(i))
    for c in (c_w2, c_w3, c_w4):
        c.wait()

    def mlp(i, c):
        def side_ops():
            half = pl.ds(pl.multiple_of(i * (_RB // 2), _RB // 2), _RB // 2)
            for t in range(D // 128):
                k = pltpu.bitcast(kbuf[t, rows(i), :], _I32)
                for j in range(hpt):
                    krot[t * hpt + j, half, :] = pltpu.roll(k, 128 - j * Dh, 1) if j else k
                    yield from range(_RB // 16)
            kv = kvf[i]
            for e in range(128):
                kbr[i * hpt + e // Dh, e % Dh] = jnp.broadcast_to(kv[:, e:e + 1], (_NV * 16, 128))
                yield from range(_NV * 2)

        nside = (D // 128) * hpt * _RB // 16 + _NV * 2 * 128
        side = side_ops()

        def advance(frac):
            for _ in range(int(nside * frac)):
                next(side, None)

        x = ax[rows(i), :]
        qv = _dot_nt(wqt[...], x) * (Dh ** -0.5 * _LOG2E)
        qf[i] = qv
        for m in range(D // 16):
            for j in range(_RB // 128):
                qt[i, m * 8:(m + 1) * 8, j * 128:(j + 1) * 128] = _pack(
                    qv[m * 16:(m + 1) * 16, j * 128:(j + 1) * 128])
        q = D // 4
        win = pl.ds(pl.multiple_of(i * _RB, _RB), _RB + 2 * _HALO)
        parts = []
        for g, sh in enumerate((1, -1, 2, -2)):
            hw = hbuf[win, g * q:(g + 1) * q]
            parts.append(hw[_HALO - sh:_HALO - sh + _RB].astype(_BF16))
        x1 = x.astype(_F32) + _dot(jnp.concatenate(parts, axis=1), w2[...])
        v = _dot_nt(wvt[...], x).astype(_BF16)
        for j in range(_RB // _KB):
            vt[i * (_RB // _KB) + j] = v[:, j * _KB:(j + 1) * _KB]
        advance(0.1)
        xn = _layernorm(x1).astype(_BF16)
        F = w3.shape[1]
        hs = []
        for n in range(0, F, _FC):
            hs.append(_gelu(_dot(xn, w3[:, n:n + _FC])).astype(_BF16))
            advance(0.5 * _FC / F)
        h = jnp.concatenate(hs, axis=1)
        ng = 1.0 - gbuf[rows(i), :]
        for n in range(0, D, _FC):
            b = x1[:, n:n + _FC] + _dot(h, w4[:, n:n + _FC])
            bbuf[rows(i), n:n + _FC] = b * jnp.concatenate([ng] * (_FC // 128), axis=1)
            advance(0.4 * _FC / D)
        for _ in side:
            pass
        return c

    jax.lax.fori_loop(0, nrb, mlp, 0)


    nq = _NQ // 128

    def q_weights(h, qb):
        return _unpack(qt[qb, pl.ds(pl.multiple_of(h * (Dh // 2), Dh // 2), Dh // 2), :])

    def head_rows(h):
        return pl.ds(pl.multiple_of(h * Dh, Dh), Dh)

    def pv(h, kb):
        return _dot(vt[kb, head_rows(h), :], _unpack(pb[kb * 64:kb * 64 + 64, :]))

    def finish_unit(h, qb, acc, l, flag):
        den = jnp.sum(l, axis=0, keepdims=True)
        ot[qb, head_rows(h), :] = (acc / den).astype(_BF16)
        return jnp.maximum(flag, jnp.where((den >= _L_LO) & (den <= _L_HI), 0.0, 1.0))

    def unit(h, qb, prev, acc, lprev, flag, zs, kslot):
        w = q_weights(h, qb)
        st = {"l": [jnp.zeros((8, 128), _F32)] * nq, "acc": acc, "flag": flag, "done": 0, "cum": 0}

        def emit(g, j, s):
            p = jnp.exp2(s)
            st["l"][j] = st["l"][j] + p[0:8] + p[8:16]
            pb[g * 8:g * 8 + 8, j * 128:(j + 1) * 128] = _pack(p)

        def vpu_ops():
            for i, g in enumerate(vset):
                qh = qf.at[qb + zs[nq + i % _ZQ], head_rows(h)]
                for j in range(nq):
                    for d in range(Dh):
                        qd = qh[d:d + 1, j * 128:(j + 1) * 128]
                        m = kbr[kslot[j], d, i * 16:i * 16 + 16, :] * qd
                        s = m if d == 0 else s + m
                        yield from range(2)
                    emit(g, j, s)
                    yield from range(2)

        work = []
        for kb in range(nkb):
            runs = []
            for g in range(kb * 8, kb * 8 + 8):
                if g in vset:
                    continue
                if runs and sum(runs[-1]) == g and (runs[-1][1] + 1) * 16 <= _RS:
                    runs[-1][1] += 1
                else:
                    runs.append([g, 1])
            work += [(False, kb - _LAG, 1)] + [(True, g, n) for g, n in runs]
        total = sum(n for _, _, n in work)
        nops = _NV * nq * (2 * Dh + 2)
        gen = vpu_ops()

        def advance(n):
            st["cum"] += n
            while st["done"] < min(nops, int(nops * st["cum"] / total)):
                next(gen)
                st["done"] += 1

        for is_qk, g, n in work:
            if is_qk:
                s = _dot(_unpack(krot[h, g * 8:(g + n) * 8, :])[:, :Dh], w)
                for r in range(n):
                    for j in range(nq):
                        emit(g + r, j, s[r * 16:r * 16 + 16, j * 128:(j + 1) * 128])
                        advance(1 / nq)
            else:
                st["acc"] = st["acc"] + pv(prev[0] if g < 0 else h, g % nkb)
                if g == -1:
                    st["flag"] = finish_unit(*prev, st["acc"], lprev, st["flag"])
                    st["acc"] = jnp.zeros((Dh, _NQ), _F32)
                advance(1)
        for _ in gen:
            pass
        return st["acc"], jnp.concatenate(st["l"], axis=1), st["flag"]

    def head(hh, flag):
        prev = (jnp.maximum(hh * _HU - 1, 0), nqb - 1)
        acc, l = accb[...], lb[...]
        zs = [zero[i] for i in range(nq + _ZQ)]
        for h in [hh * _HU + i for i in range(_HU)]:
            kslot = [h + zs[j] for j in range(nq)]
            for qb in range(nqb):
                acc, l, flag = unit(h, qb, prev, acc, l, flag, zs, kslot)
                prev = (h, qb)
        accb[...] = acc
        lb[...] = l
        return flag

    flag = jax.lax.fori_loop(0, _H // _HU, head, jnp.zeros((1, _NQ), _F32))
    onat = (wq, wk, wv, w1)

    def untranspose(i):
        onat[i][...] = ot[i].T

    c_wo.wait()
    for i in range(2):
        untranspose(i)
    acc = accb[...]
    for kb in range(nkb - _LAG, nkb):
        acc = acc + pv(_H - 1, kb)
    flag = finish_unit(_H - 1, nqb - 1, acc, lb[...], flag)

    def project(chunks, pending):
        copies = []
        chk = jnp.zeros((8, 128), _F32)
        for n, (r0, nr) in enumerate(chunks):
            r = slice(r0, r0 + nr)
            if n == 0:
                for i in pending:
                    untranspose(i)
            o = onat[r0 // _NQ][r0 % _NQ:r0 % _NQ + nr, :]
            g = jnp.concatenate([gbuf[r, :]] * (D // 128), axis=1)
            a = _dot(o, wo[...])
            ax[r, :] = (g * a + bbuf[r, :]).astype(ax.dtype)
            chk = chk + jnp.sum((a[:, :128] * 0.0).reshape(nr // 8, 8, 128), axis=0)
            copies.append(pltpu.make_async_copy(ax.at[r], out_hbm.at[r], osems.at[n]))
            copies[-1].start()
            if n:
                copies[-2].wait()
        copies[-1].wait()
        return chk

    chk = project([(r0, _NQ) for r0 in range(0, S - _NQ, _NQ)]
            + [(S - _NQ, _NQ - _LC), (S - _LC, _LC)], range(2, nqb))

    worst = jnp.maximum(jnp.max(flag), jnp.max(jnp.where(chk == 0.0, 0.0, 1.0)))

    @pl.when(worst > 0.0)
    def _():
        def safe_unit(u, c):
            h = jax.lax.div(u, nqb)
            w = q_weights(h, jax.lax.rem(u, nqb))
            hr = head_rows(h)

            def scores(kb):
                k = krot[h, pl.ds(pl.multiple_of(kb * 64, 64), 64), :]
                return _dot(_unpack(k)[:, :Dh], w)

            m = jax.lax.fori_loop(
                0, nkb, lambda kb, m: jnp.maximum(m, jnp.max(scores(kb), axis=0, keepdims=True)),
                jnp.full((1, _NQ), -jnp.inf, _F32))

            def accum(kb, carry):
                den, acc = carry
                p = jnp.exp2(scores(kb) - m)
                return (den + jnp.sum(p, axis=0, keepdims=True),
                        acc + _dot(vt[kb, hr, :], p.astype(_BF16)))

            den, acc = jax.lax.fori_loop(
                0, nkb, accum, (jnp.zeros((1, _NQ), _F32), jnp.zeros((Dh, _NQ), _F32)))
            ot[jax.lax.rem(u, nqb), hr, :] = (acc / den).astype(_BF16)
            return c

        jax.lax.fori_loop(0, _H * nqb, safe_unit, 0)
        project([(r0, _NQ) for r0 in range(0, S, _NQ)], range(nqb))


@jax.jit
def pallas_gated_mix__mha_block__mixer_s_mlp__prompt_kernel(
    A_x: jax.Array,
    A_wqkv: jax.Array,
    A_wo: jax.Array,
    B_x: jax.Array,
    B_w1: jax.Array,
    B_w2: jax.Array,
    B_w3: jax.Array,
    B_w4: jax.Array,
    gate_w: jax.Array,
):
    del B_x
    B, S, D = A_x.shape
    F = B_w3.shape[1]
    assert B == 1
    vm = pltpu.VMEM
    sq = vm((D, D), _BF16)
    scratch = [
        vm((S, D), _BF16), sq, sq, sq, sq, sq, sq,
        vm((D, F), _BF16), vm((F, D), _BF16), vm((D,), _BF16),
        vm((S + 2 * _HALO, D), _F32),
        vm((S, D), _F32),
        vm((S, 128), _F32),
        sq, sq,
        vm((D // 128, S, 128), _BF16),
        vm((D // 128, _NV * 16, 128), _F32),
        vm((_H, S // 2, 128), _I32),
        vm((_H, D // _H, _NV * 16, 128), _F32),
        vm((S // _NQ, D // 2, _NQ), _I32),
        vm((S // _NQ, D, _NQ), _F32),
        vm((S // _KB, D, _KB), _BF16),
        vm((S // _NQ, D, _NQ), _BF16),
        vm((S // 2, _NQ), _I32),
        vm((D // _H, _NQ), _F32), vm((8, _NQ), _F32),
        pltpu.SMEM((_NQ // 128 + _ZQ,), _I32),
        pltpu.SemaphoreType.DMA((9,)),
        pltpu.SemaphoreType.DMA((S // _RB,)),
        pltpu.SemaphoreType.DMA((S // _NQ + 1,)),
    ]
    out = pl.pallas_call(
        _kernel,
        out_shape=jax.ShapeDtypeStruct((S, D), A_x.dtype),
        in_specs=[pl.BlockSpec(memory_space=pl.ANY)] * 8,
        out_specs=pl.BlockSpec(memory_space=pl.ANY),
        scratch_shapes=scratch,
        compiler_params=pltpu.CompilerParams(
            vmem_limit_bytes=124 * 1024 * 1024,
            flags={"XLA_TPU_FORCE_LP_LLO_SCHEDULER": True}),
    )(A_x.reshape(S, D), A_wqkv, A_wo, B_w1, B_w2, B_w3, B_w4, gate_w)
    return out.reshape(B, S, D)
```
